```python
import os as _os
_os.environ.setdefault("JAX_PLATFORMS", "cpu")
import jax
import jax.numpy as jnp

def _softmax(x, axis=-1):
    return jax.nn.softmax(x, axis=axis)
def _gelu(x):
    return jax.nn.gelu(x, approximate=True)
def _silu(x):
    return jax.nn.silu(x)
def _sigmoid(x):
    return jax.nn.sigmoid(x)
def _layernorm(x, axis=-1, eps=1e-5):
    m = jnp.mean(x, axis=axis, keepdims=True)
    v = jnp.var(x, axis=axis, keepdims=True)
    return (x - m) / jnp.sqrt(v + eps)
def _scatter_add(tgt, idx, src, axis=0):
    return tgt.at[idx].add(src)
def _segment_sum(src, seg, n):
    return jax.ops.segment_sum(src, seg, n)
class _Rng:
    def __init__(self, key):
        self._k = key
    def _next(self):
        self._k, sub = jax.random.split(self._k)
        return sub
    def normal(self, shape):
        return jax.random.normal(self._next(), shape, dtype=jnp.bfloat16)
    def randint(self, lo, hi, shape):
        return jax.random.randint(self._next(), shape, lo, hi, dtype=jnp.int32)
    def uniform(self, shape, lo=0.0, hi=1.0):
        return jax.random.uniform(self._next(), shape, jnp.bfloat16, lo, hi)
    def permutation(self, n):
        return jax.random.permutation(self._next(), n)


kernel_name = 'standalone__mha_softmax__near_ridge'

def setup_inputs():
    _rng = _Rng(jax.random.key(int.from_bytes(__import__("os").urandom(4), "little")))
    _w = (lambda a: (lambda t: t.astype(jnp.bfloat16) if jnp.issubdtype(t.dtype, jnp.floating) else t)(jnp.asarray(a)))
    B, H, Sq, Sk, D = 8, 32, 304, 2048, 128
    return {
        "q": _w((lambda *s: _rng.normal(s) * 0.4)(B, H, Sq, D)),
        "k": _w((lambda *s: _rng.normal(s) * 0.4)(B, H, Sk, D)),
        "v": _w((lambda *s: _rng.normal(s) * 0.05)(B, H, Sk, D)),
    }

def reference(q, k, v):
    scale = q.shape[-1] ** -0.5
    scores = jnp.einsum("bhqd,bhkd->bhqk", q, k) * scale
    p = _softmax(scores, axis=-1)
    return jnp.einsum("bhqk,bhkd->bhqd", p, v)
```

```python
import functools
import jax
import jax.numpy as jnp
from jax import lax
import jax.experimental.pallas as pl
import jax.experimental.pallas.tpu as pltpu

HB = 8

@jax.jit
def pallas_standalone__mha_softmax__near_ridge_kernel(q, k, v):
    B, H, Sq, D = q.shape
    Sk = k.shape[2]
    BH = B * H
    scale = float(D) ** -0.5
    q3 = q.reshape(BH, Sq, D)
    k3 = k.reshape(BH, Sk, D)
    v3 = v.reshape(BH, Sk, D)

    def kernel(q_ref, k_ref, v_ref, o_ref):
        for h in range(HB):
            qh = q_ref[h]
            kh = k_ref[h]
            vh = v_ref[h]
            s = lax.dot_general(qh, kh, (((1,), (1,)), ((), ())),
                                preferred_element_type=jnp.float32)
            m = jnp.max(s, axis=-1, keepdims=True)
            p = jnp.exp((s - m) * scale)
            l = jnp.sum(p, axis=-1, keepdims=True)
            o = jnp.dot(p.astype(jnp.bfloat16), vh, preferred_element_type=jnp.float32)
            o_ref[h] = (o / l).astype(o_ref.dtype)

    out = pl.pallas_call(
        kernel,
        grid=(BH // HB,),
        in_specs=[
            pl.BlockSpec((HB, Sq, D), lambda i: (i, 0, 0)),
            pl.BlockSpec((HB, Sk, D), lambda i: (i, 0, 0)),
            pl.BlockSpec((HB, Sk, D), lambda i: (i, 0, 0)),
        ],
        out_specs=pl.BlockSpec((HB, Sq, D), lambda i: (i, 0, 0)),
        out_shape=jax.ShapeDtypeStruct((BH, Sq, D), q.dtype),
        compiler_params=pltpu.CompilerParams(
            dimension_semantics=("arbitrary",),
            vmem_limit_bytes=100 * 1024 * 1024,
        ),
    )(q3, k3, v3)
    return out.reshape(B, H, Sq, D)
```

```python
import math

import jax
import jax.numpy as jnp
from jax import lax
import jax.experimental.pallas as pl
import jax.experimental.pallas.tpu as pltpu

_HEADS_PER_STEP = 8


@jax.jit
def pallas_standalone__mha_softmax__near_ridge_kernel(
    q: jax.Array,
    k: jax.Array,
    v: jax.Array,
):
    B, H, Sq, D = q.shape
    Sk = k.shape[2]
    BH = B * H
    hb = _HEADS_PER_STEP if BH % _HEADS_PER_STEP == 0 else 1
    c = (float(D) ** -0.5) * math.log2(math.e)

    q3 = q.reshape(BH, Sq, D)
    k3 = k.reshape(BH, Sk, D)
    v3 = v.reshape(BH, Sk, D)

    def kernel(q_ref, k_ref, v_ref, o_ref):
        for h in range(hb):
            qh = (q_ref[h].astype(jnp.float32) * c).astype(jnp.bfloat16)
            s = lax.dot_general(qh, k_ref[h], (((1,), (1,)), ((), ())),
                                preferred_element_type=jnp.float32)
            m = jnp.max(s, axis=-1, keepdims=True)
            p = jnp.exp2(s - m)
            l = jnp.sum(p, axis=-1, keepdims=True)
            r = pl.reciprocal(l, approx=True)
            r = r * (2.0 - l * r)
            o = jnp.dot(p.astype(jnp.bfloat16), v_ref[h],
                        preferred_element_type=jnp.float32)
            o_ref[h] = (o * r).astype(o_ref.dtype)

    out = pl.pallas_call(
        kernel,
        grid=(BH // hb,),
        in_specs=[
            pl.BlockSpec((hb, Sq, D), lambda i: (i, 0, 0)),
            pl.BlockSpec((hb, Sk, D), lambda i: (i, 0, 0)),
            pl.BlockSpec((hb, Sk, D), lambda i: (i, 0, 0)),
        ],
        out_specs=pl.BlockSpec((hb, Sq, D), lambda i: (i, 0, 0)),
        out_shape=jax.ShapeDtypeStruct((BH, Sq, D), q.dtype),
        compiler_params=pltpu.CompilerParams(
            dimension_semantics=("arbitrary",),
            vmem_limit_bytes=100 * 1024 * 1024,
            disable_bounds_checks=True,
        ),
    )(q3, k3, v3)
    return out.reshape(B, H, Sq, D)
```
